```python
import os as _os
_os.environ.setdefault("JAX_PLATFORMS", "cpu")
import jax
import jax.numpy as jnp

def _softmax(x, axis=-1):
    return jax.nn.softmax(x, axis=axis)
def _gelu(x):
    return jax.nn.gelu(x, approximate=True)
def _silu(x):
    return jax.nn.silu(x)
def _sigmoid(x):
    return jax.nn.sigmoid(x)
def _layernorm(x, axis=-1, eps=1e-5):
    m = jnp.mean(x, axis=axis, keepdims=True)
    v = jnp.var(x, axis=axis, keepdims=True)
    return (x - m) / jnp.sqrt(v + eps)
def _scatter_add(tgt, idx, src, axis=0):
    return tgt.at[idx].add(src)
def _segment_sum(src, seg, n):
    return jax.ops.segment_sum(src, seg, n)
class _Rng:
    def __init__(self, key):
        self._k = key
    def _next(self):
        self._k, sub = jax.random.split(self._k)
        return sub
    def normal(self, shape):
        return jax.random.normal(self._next(), shape, dtype=jnp.bfloat16)
    def randint(self, lo, hi, shape):
        return jax.random.randint(self._next(), shape, lo, hi, dtype=jnp.int32)
    def uniform(self, shape, lo=0.0, hi=1.0):
        return jax.random.uniform(self._next(), shape, jnp.bfloat16, lo, hi)
    def permutation(self, n):
        return jax.random.permutation(self._next(), n)


kernel_name = 'concat_heads__gqa_block_cached__sliding_block_cached__decode'

def setup_inputs():
    _rng = _Rng(jax.random.key(int.from_bytes(__import__("os").urandom(4), "little")))
    _w = (lambda a: (lambda t: t.astype(jnp.bfloat16) if jnp.issubdtype(t.dtype, jnp.floating) else t)(jnp.asarray(a)))
    def _A_setup():
        B, Sq, D = 2, 1, 448
        Hq, Hkv, Sk, Dh = 16, 8, 8192, 256
        assert Hq % Hkv == 0, (Hq, Hkv)
        return {
            "x": _w((lambda *s: _rng.normal(s) * 0.8)(B, Sq, D)),
            "k_cache": _w((lambda *s: _rng.normal(s) * 0.8)(B, Hkv, Sk, Dh)),
            "v_cache": _w((lambda *s: _rng.normal(s) * 0.05)(B, Hkv, Sk, Dh)),
            "wq": _w((lambda *s: _rng.normal(s) * 0.8)(D, Hq * Dh) * (D ** -0.5)),
            "wo": _w((lambda *s: _rng.normal(s) * 0.05)(Hq * Dh, D) * ((Hq * Dh) ** -0.5)),
        }
    _A_in = _A_setup()

    def _B_setup():
        B, Sq, D = 2, 1, 448
        Hq, Hkv, Sk, Dh = 16, 8, 8192, 256
        assert Hq % Hkv == 0, (Hq, Hkv)
        return {
            "x": _w((lambda *s: _rng.normal(s) * 0.8)(B, Sq, D)),
            "k_cache": _w((lambda *s: _rng.normal(s) * 0.8)(B, Hkv, Sk, Dh)),
            "v_cache": _w((lambda *s: _rng.normal(s) * 0.05)(B, Hkv, Sk, Dh)),
            "wq": _w((lambda *s: _rng.normal(s) * 0.8)(D, Hq * Dh) * (D ** -0.5)),
            "wo": _w((lambda *s: _rng.normal(s) * 0.05)(Hq * Dh, D) * ((Hq * Dh) ** -0.5)),
        }
    _B_in = _B_setup()

    return {
        "A_x": _A_in["x"],
        "A_k_cache": _A_in["k_cache"],
        "A_v_cache": _A_in["v_cache"],
        "A_wq": _A_in["wq"],
        "A_wo": _A_in["wo"],
        "B_x": _B_in["x"],
        "B_k_cache": _B_in["k_cache"],
        "B_v_cache": _B_in["v_cache"],
        "B_wq": _B_in["wq"],
        "B_wo": _B_in["wo"],
    }

def reference(A_x, A_k_cache, A_v_cache, A_wq, A_wo, B_x, B_k_cache, B_v_cache, B_wq, B_wo):
    def _A_ref(x, k_cache, v_cache, wq, wo):
        B, Sq, D = x.shape
        Hq, Dh = 16, 256
        Hkv = k_cache.shape[1]
        rep = Hq // Hkv
        q = (lambda x, *d: x.transpose(*d))((x @ wq).reshape(B, Sq, Hq, Dh), 0, 2, 1, 3)
        k = jnp.repeat(k_cache, rep, axis=1)
        v = jnp.repeat(v_cache, rep, axis=1)
        scores = jnp.einsum("bhqd,bhkd->bhqk", q, k) * (Dh ** -0.5)
        p = _softmax(scores, axis=-1)
        o = jnp.einsum("bhqk,bhkd->bhqd", p, v)
        return (lambda x, *d: x.transpose(*d))(o, 0, 2, 1, 3).reshape(B, Sq, Hq * Dh) @ wo

    def _B_ref(x, k_cache, v_cache, wq, wo):
        B, Sq, D = x.shape
        Hq, Dh = 16, 256
        Hkv, Sk = k_cache.shape[1], k_cache.shape[2]
        W = min(4096, max(256, Sk // 4))
        rep = Hq // Hkv
        q = (lambda x, *d: x.transpose(*d))((x @ wq).reshape(B, Sq, Hq, Dh), 0, 2, 1, 3)
        k = jnp.repeat(k_cache[:, :, Sk - W:, :], rep, axis=1)
        v = jnp.repeat(v_cache[:, :, Sk - W:, :], rep, axis=1)
        scores = jnp.einsum("bhqd,bhkd->bhqk", q, k) * (Dh ** -0.5)
        p = _softmax(scores, axis=-1)
        o = jnp.einsum("bhqk,bhkd->bhqd", p, v)
        return (lambda x, *d: x.transpose(*d))(o, 0, 2, 1, 3).reshape(B, Sq, Hq * Dh) @ wo

    a = _A_ref(A_x, A_k_cache, A_v_cache, A_wq, A_wo)
    b = _B_ref(B_x, B_k_cache, B_v_cache, B_wq, B_wo)
    return jnp.concatenate([a, b], axis=-1)
```

```python
import functools
import jax
import jax.numpy as jnp
from jax import lax
import jax.experimental.pallas as pl
import jax.experimental.pallas.tpu as pltpu

B, D, HQ, HKV, DH = 2, 448, 16, 8, 256
HD = HQ * DH
LOG2E = 1.4426950408889634
NT = (((1,), (1,)), ((), ()))


def make(R=2048, LOOK=3, C=64, TK=256, mode="after", swap=0, nobc=True, nocompute=False):
    NBUF = LOOK + 1
    NP = R // C
    WC = 2048
    WP = (D // 8) * (HD // WC)
    NTILE = R // TK

    def kernel(ax, ak, av, awq, awo, bx, bk, bv, bwq, bwo, out,
               kv, x_buf, wq_buf, wo_buf, q_scr, o_scr, kv_sem, x_sem, wq_sem, wo_sem):
        SK = ak.shape[0] // (B * HKV)
        W = min(4096, max(256, SK // 4))
        nA, nB = SK // R, W // R
        stepsA, stepsB = B * HKV * nA, B * HKV * nB
        steps = stepsA + stepsB

        def kv_starts(k, v, base, slot):
            def one(j):
                def go():
                    src = pl.ds(pl.multiple_of(base + j * C, C), C)
                    pltpu.make_async_copy(k.at[src], kv.at[slot, 0, pl.ds(j * C, C)], kv_sem.at[slot]).start(priority=swap)
                    pltpu.make_async_copy(v.at[src], kv.at[slot, 1, pl.ds(j * C, C)], kv_sem.at[slot]).start(priority=1 - swap)
                return go
            return [one(j) for j in range(NP)]

        def w_start(srcs, buf, semf, j):
            per = HD // WC
            r = j // per
            c = j % per
            if not isinstance(j, int):
                r8 = pl.multiple_of(r * 8, 8)
                c0 = pl.multiple_of(c * WC, WC)
            else:
                r8, c0 = r * 8, c * WC
            for i in range(2):
                pltpu.make_async_copy(srcs[i].at[pl.ds(r8, 8), pl.ds(c0, WC)], buf.at[i, pl.ds(r8, 8), pl.ds(c0, WC)], semf(i, r)).start(priority=i ^ swap)

        wq_start = functools.partial(w_start, (awq, bwq), wq_buf, lambda i, r: wq_sem.at[i])
        wo_start = functools.partial(w_start, (awo, bwo), wo_buf, lambda i, r: wo_sem.at[i * 4 + r // 16])

        def baseB(u):
            return (u // nB) * SK + (SK - W) + (u % nB) * R

        wq_start(0)
        x_copies = [pltpu.make_async_copy(x, x_buf.at[i], x_sem.at[i]) for i, x in enumerate((ax, bx))]
        for c in x_copies:
            c.start()
        lax.fori_loop(1, WP, lambda j, _: wq_start(j), None, unroll=3)

        def pro(t, _):
            for g in kv_starts(ak, av, t * R, t):
                g()
        lax.fori_loop(0, LOOK - 1, pro, None)

        row = lax.broadcasted_iota(jnp.int32, (8, DH), 0)
        o_scr[...] = jnp.zeros(o_scr.shape, o_scr.dtype)
        pend = kv_starts(ak, av, (LOOK - 1) * R, LOOK - 1)
        per = NP // (2 * HKV)
        for i in range(2):
            x_copies[i].wait()
            xf = x_buf[i].astype(jnp.float32)
            xr = lax.broadcasted_iota(jnp.int32, (8, D), 0)
            x8 = jnp.where(xr % 2 == 0, xf[0:1, :], xf[1:2, :]).astype(jnp.bfloat16)
            pltpu.make_async_copy(wq_buf.at[i], wq_buf.at[i], wq_sem.at[i]).wait()
            for h in range(HKV):
                q2 = jnp.dot(x8, wq_buf[i, :, h * 2 * DH:(h + 1) * 2 * DH], preferred_element_type=jnp.float32)
                q_scr[i * HKV + h] = jnp.where(row < 2, q2[:, :DH], q2[:, DH:])
                for _ in range(per):
                    pend.pop(0)()
        assert not pend

        def step(starts_fn, t, carry):
            m, l, acc = carry
            slot = t % NBUF
            pend = starts_fn(t + LOOK, (t + LOOK) % NBUF)
            npend = len(pend)
            def issue(upto):
                while len(pend) > npend - upto * npend // (2 * NTILE):
                    pend.pop(0)()
            isA = t < stepsA
            tt = jnp.where(isA, t, t - stepsA)
            bh = jnp.where(isA, tt // nA, tt // nB)
            c = jnp.where(isA, tt % nA, tt % nB)
            last = c == jnp.where(isA, nA - 1, nB - 1)
            b = bh // HKV
            hidx = bh % HKV + jnp.where(isA, 0, HKV)
            first = c == 0
            m = jnp.where(first, -jnp.inf, m)
            l = jnp.where(first, 0.0, l)
            acc = jnp.where(first, 0.0, acc)
            q = q_scr[hidx].astype(jnp.bfloat16)
            pltpu.make_async_copy(kv.at[slot], kv.at[slot], kv_sem.at[slot]).wait()
            if nocompute:
                issue(2 * NTILE)
                return m, l, acc
            if mode == "before":
                issue(2 * NTILE)
            ss = []
            for j in range(NTILE):
                ss.append(lax.dot_general(q, kv[slot, 0, j * TK:(j + 1) * TK, :], NT, preferred_element_type=jnp.float32))
                if mode == "inter":
                    issue(j + 1)
            s = jnp.concatenate(ss, axis=1) * (LOG2E * DH ** -0.5)
            m_new = jnp.maximum(m, jnp.max(s, axis=1, keepdims=True))
            alpha = jnp.exp2(m - m_new)
            p = jnp.exp2(s - m_new)
            l = l * alpha + jnp.sum(p, axis=1, keepdims=True)
            pb = p.astype(jnp.bfloat16)
            acc = acc * alpha
            for j in range(NTILE):
                acc = acc + jnp.dot(pb[:, j * TK:(j + 1) * TK], kv[slot, 1, j * TK:(j + 1) * TK, :], preferred_element_type=jnp.float32)
                if mode == "inter":
                    issue(NTILE + j + 1)
            issue(2 * NTILE)
            keep = jnp.logical_and(row % 2 == b, last)
            o_scr[hidx] = jnp.where(keep, acc / l, o_scr[hidx])
            return m_new, l, acc

        carry = (jnp.zeros((8, 1), jnp.float32), jnp.zeros((8, 1), jnp.float32), jnp.zeros((8, DH), jnp.float32))
        carry = lax.fori_loop(0, stepsA - LOOK, functools.partial(step, lambda u, s: kv_starts(ak, av, u * R, s)), carry)
        carry = lax.fori_loop(stepsA - LOOK, steps - LOOK, functools.partial(step, lambda u, s: kv_starts(bk, bv, baseB(u - stepsA), s)), carry)
        assert LOOK * NP <= WP
        carry = lax.fori_loop(steps - LOOK, steps, functools.partial(
            step, lambda u, s: [functools.partial(wo_start, (u - steps) * NP + j) for j in range(NP)]), carry)

        pend = [functools.partial(wo_start, j) for j in range(LOOK * NP, WP)]
        lhs = []
        for i in range(2):
            parts = []
            for hq in range(HQ):
                oh = o_scr[i * HKV + hq // 2]
                parts.append(jnp.where(row // 2 == hq % 2, oh, 0.0).astype(jnp.bfloat16))
            lhs.append(parts)
        res = [[], []]
        KP = 4
        for g in range(4):
            r0, r1 = g * 128, min(D, (g + 1) * 128)
            if g == 2:
                while pend:
                    pend.pop(0)()
            for i in range(2):
                dst = wo_buf.at[i, pl.ds(r0, r1 - r0)]
                pltpu.make_async_copy(dst, dst, wo_sem.at[i * 4 + g]).wait()
                r = None
                for c in range(HQ // KP):
                    d = lax.dot_general(jnp.concatenate(lhs[i][c * KP:(c + 1) * KP], axis=1),
                                        wo_buf[i, r0:r1, c * KP * DH:(c + 1) * KP * DH], NT, preferred_element_type=jnp.float32)
                    r = d if r is None else r + d
                    for _ in range(2):
                        if pend:
                            pend.pop(0)()
                res[i].append(r[0:2] + r[2:4])
        out[...] = jnp.concatenate(res[0] + res[1], axis=1).astype(out.dtype)

    def f(A_x, A_k_cache, A_v_cache, A_wq, A_wo, B_x, B_k_cache, B_v_cache, B_wq, B_wo):
        hbm = pl.BlockSpec(memory_space=pltpu.HBM)
        out = pl.pallas_call(
            kernel,
            out_shape=jax.ShapeDtypeStruct((B, 2 * D), jnp.bfloat16),
            in_specs=[hbm] * 10,
            out_specs=pl.BlockSpec(memory_space=pltpu.VMEM),
            scratch_shapes=[
                pltpu.VMEM((NBUF, 2, R, DH), jnp.bfloat16),
                pltpu.VMEM((2, B, D), jnp.bfloat16),
                pltpu.VMEM((2, D, HD), jnp.bfloat16),
                pltpu.VMEM((2, D, HD), jnp.bfloat16),
                pltpu.VMEM((2 * HKV, 8, DH), jnp.float32),
                pltpu.VMEM((2 * HKV, 8, DH), jnp.float32),
                pltpu.SemaphoreType.DMA((NBUF,)),
                pltpu.SemaphoreType.DMA((2,)),
                pltpu.SemaphoreType.DMA((2,)),
                pltpu.SemaphoreType.DMA((8,)),
            ],
            compiler_params=pltpu.CompilerParams(vmem_limit_bytes=100 * 2**20, disable_bounds_checks=nobc),
        )(A_x.reshape(B, D), A_k_cache.reshape(-1, DH), A_v_cache.reshape(-1, DH), A_wq, A_wo.T,
          B_x.reshape(B, D), B_k_cache.reshape(-1, DH), B_v_cache.reshape(-1, DH), B_wq, B_wo.T)
        return out.reshape(B, 1, 2 * D)
    return f


@jax.jit
def pallas_concat_heads__gqa_block_cached__sliding_block_cached__decode_kernel(
    A_x, A_k_cache, A_v_cache, A_wq, A_wo, B_x, B_k_cache, B_v_cache, B_wq, B_wo):
    return make()(A_x, A_k_cache, A_v_cache, A_wq, A_wo, B_x, B_k_cache, B_v_cache, B_wq, B_wo)
```

```python
import functools
import jax
import jax.numpy as jnp
from jax import lax
import jax.experimental.pallas as pl
import jax.experimental.pallas.tpu as pltpu

B, D, HQ, HKV, DH = 2, 448, 16, 8, 256
HD = HQ * DH
LOG2E = 1.4426950408889634
NT = (((1,), (1,)), ((), ()))
C = 64
WC = 2048
R = 2048


def make(LOOK=4, NBUF=6, KA=4, WQS=7, mode="after", swap=0, nobc=True, nosem=False, nocompute=False, noproj=False, tail=2, flags=None):
    wo_blocks = []
    groups = []
    for j in range(8):
        for c in range(2):
            for m in range(4):
                wo_blocks.append((m * 64 + j * 8, c * WC, m // 2))
    for j in range(8):
        for c in range(2):
            for m in range(2):
                wo_blocks.append((256 + m * 64 + j * 8, c * WC, 2))
    groups = [(0, 128, 0, HD), (128, 256, 0, HD), (256, 384, 0, HD)]
    if tail == 1:
        for j in range(8):
            for c in range(2):
                wo_blocks.append((384 + j * 8, c * WC, 3))
        groups += [(384, 448, 0, HD)]
    else:
        for c in range(2):
            for j in range(8):
                wo_blocks.append((384 + j * 8, c * WC, 3 + c))
        groups += [(384, 448, 0, WC), (384, 448, WC, HD)]
    NG = len(groups)
    NW1 = 64 // LOOK

    def kernel(ax, ak, av, awq, awo, bx, bk, bv, bwq, bwo, out,
               kv, x_buf, wq_buf, wo_buf, q_scr, o_scr, kv_sem, x_sem, wq_sem, wo_sem):
        SK = ak.shape[0] // (B * HKV)
        W = min(4096, max(256, SK // 4))
        nA, nB = SK // R, W // R
        assert nB == 1
        stepsA, stepsB = B * HKV * nA, B * HKV * nB
        steps = stepsA + stepsB

        def al(x, n):
            return x if isinstance(x, int) else pl.multiple_of(x, n)

        def kv_pair(k, v, src, slot, dst):
            src, dst = pl.ds(al(src, C), C), pl.ds(al(dst, C), C)
            pltpu.make_async_copy(k.at[src], kv.at[slot, 0, dst], kv_sem.at[slot]).start(priority=swap)
            pltpu.make_async_copy(v.at[src], kv.at[slot, 1, dst], kv_sem.at[slot]).start(priority=1 - swap)

        def startA(u, part=(0, 1)):
            seg = R // KA
            base = (u // nA) * SK + (u % nA) * seg
            n = seg // C
            for i in range(part[0] * n // part[1], (part[0] + 1) * n // part[1]):
                for m in range(KA):
                    kv_pair(ak, av, base + m * (SK // KA) + i * C, u % NBUF, m * seg + i * C)

        def startB(u):
            ub = u - stepsA
            first = ub - ub % 2
            half = (ub % 2) * (R // 4)
            slots = [(first + e + stepsA) % NBUF for e in range(2)]
            for i in range(R // 4 // C):
                for e in range(2):
                    for m in range(2):
                        r = m * (R // 2) + i * C + half
                        kv_pair(bk, bv, (first + e) * SK + (SK - W) + r, slots[e], r)

        def w_pair(srcs, buf, sems, r, c):
            rows, cols = pl.ds(al(r, 8), 8), pl.ds(c, WC)
            for i in range(2):
                pltpu.make_async_copy(srcs[i].at[rows, cols], buf.at[i, rows, cols], sems[i]).start(priority=i ^ swap)

        def wq_start(j):
            for c in range(2):
                for m in range(WQS):
                    w_pair((awq, bwq), wq_buf, (wq_sem.at[0], wq_sem.at[1]), m * (D // WQS) + j * 8, c * WC)

        def wo_pair(r, c, g):
            w_pair((awo, bwo), wo_buf, (wo_sem.at[g], wo_sem.at[NG + g]), r, c)

        wq_start(0)
        x_copies = [pltpu.make_async_copy(x, x_buf.at[i], x_sem.at[i]) for i, x in enumerate((ax, bx))]
        for c in x_copies:
            c.start()
        lax.fori_loop(1, D // WQS // 8, lambda j, _: wq_start(j), None)
        lax.fori_loop(0, LOOK - 2, lambda t, _: startA(t), None)

        row = lax.broadcasted_iota(jnp.int32, (8, DH), 0)
        o_scr[...] = jnp.zeros(o_scr.shape, o_scr.dtype)
        for i in range(2):
            x_copies[i].wait()
            xf = x_buf[i].astype(jnp.float32)
            xr = lax.broadcasted_iota(jnp.int32, (8, D), 0)
            x8 = jnp.where(xr % 2 == 0, xf[0:1, :], xf[1:2, :]).astype(jnp.bfloat16)
            pltpu.make_async_copy(wq_buf.at[i], wq_buf.at[i], wq_sem.at[i]).wait()
            def q_head(h):
                cols = pl.ds(al(h * 2 * DH, 2 * DH), 2 * DH)
                q2 = jnp.dot(x8, wq_buf[i, :, cols], preferred_element_type=jnp.float32)
                q_scr[i * HKV + h] = jnp.where(row < 2, q2[:, :DH], q2[:, DH:])
            for half in range(2):
                lax.fori_loop(half * 4, half * 4 + 4, lambda h, _: q_head(h), None)
                startA(LOOK - 2 + i, (half, 2))

        def step(start_fn, t, carry):
            m, l, acc = carry
            slot = t % NBUF
            isA = t < stepsA
            bh = jnp.where(isA, t // nA, t - stepsA)
            c = jnp.where(isA, t % nA, 0)
            last = c == jnp.where(isA, nA - 1, 0)
            b = bh // HKV
            hidx = bh % HKV + jnp.where(isA, 0, HKV)
            first = c == 0
            m = jnp.where(first, -jnp.inf, m)
            l = jnp.where(first, 0.0, l)
            acc = jnp.where(first, 0.0, acc)
            q = q_scr[hidx].astype(jnp.bfloat16)
            pltpu.make_async_copy(kv.at[slot], kv.at[slot], kv_sem.at[slot]).wait()
            if nocompute:
                start_fn(t + LOOK)
                return m, l, acc
            if mode == "before":
                start_fn(t + LOOK)
            s = lax.dot_general(q, kv[slot, 0], NT, preferred_element_type=jnp.float32) * (LOG2E * DH ** -0.5)
            if mode == "mid":
                start_fn(t + LOOK)
            m_new = jnp.maximum(m, jnp.max(s, axis=1, keepdims=True))
            alpha = jnp.exp2(m - m_new)
            p = jnp.exp2(s - m_new)
            l = l * alpha + jnp.sum(p, axis=1, keepdims=True)
            acc = acc * alpha + jnp.dot(p.astype(jnp.bfloat16), kv[slot, 1], preferred_element_type=jnp.float32)
            if mode == "after":
                start_fn(t + LOOK)
            keep = jnp.logical_and(row % 2 == b, last)
            o_scr[hidx] = jnp.where(keep, acc / l, o_scr[hidx])
            return m_new, l, acc

        def startW(u):
            per_j = NW1 // 8
            for jj in range(per_j):
                r = ((u - steps) * per_j + jj) * 8
                for c in range(2):
                    for m in range(4):
                        wo_pair(m * 64 + r, c * WC, m // 2)

        carry = (jnp.zeros((8, 1), jnp.float32), jnp.zeros((8, 1), jnp.float32), jnp.zeros((8, DH), jnp.float32))
        carry = lax.fori_loop(0, stepsA - LOOK, functools.partial(step, startA), carry)
        carry = lax.fori_loop(stepsA - LOOK, steps - LOOK, functools.partial(step, startB), carry)
        carry = lax.fori_loop(steps - LOOK, steps, functools.partial(step, startW), carry)

        for blk in wo_blocks[LOOK * (NW1 // 8) * 8:]:
            wo_pair(*blk)
        lhs = []
        for i in range(2):
            parts = []
            for hq in range(HQ):
                oh = o_scr[i * HKV + hq // 2]
                parts.append(jnp.where(row // 2 == hq % 2, oh, 0.0).astype(jnp.bfloat16))
            lhs.append(jnp.concatenate(parts, axis=1))
        res = [{}, {}]
        for g, (r0, r1, c0, c1) in enumerate(groups):
            for i in range(2):
                dst = wo_buf.at[i, pl.ds(r0, r1 - r0), pl.ds(c0, c1 - c0)]
                pltpu.make_async_copy(dst, dst, wo_sem.at[i * NG + g]).wait()
                if noproj:
                    res[i][r0] = jnp.zeros((8, r1 - r0), jnp.float32)
                    continue
                r = lax.dot_general(lhs[i][:, c0:c1], wo_buf[i, r0:r1, c0:c1], NT, preferred_element_type=jnp.float32)
                res[i][r0] = res[i][r0] + r if r0 in res[i] else r
        out[...] = jnp.concatenate([r[0:2] + r[2:4] for i in range(2) for r in res[i].values()], axis=1).astype(out.dtype)

    def f(A_x, A_k_cache, A_v_cache, A_wq, A_wo, B_x, B_k_cache, B_v_cache, B_wq, B_wo):
        hbm = pl.BlockSpec(memory_space=pltpu.HBM)
        out = pl.pallas_call(
            kernel,
            out_shape=jax.ShapeDtypeStruct((B, 2 * D), jnp.bfloat16),
            in_specs=[hbm] * 10,
            out_specs=pl.BlockSpec(memory_space=pltpu.VMEM),
            scratch_shapes=[
                pltpu.VMEM((NBUF, 2, R, DH), jnp.bfloat16),
                pltpu.VMEM((2, B, D), jnp.bfloat16),
                pltpu.VMEM((2, D, HD), jnp.bfloat16),
                pltpu.VMEM((2, D, HD), jnp.bfloat16),
                pltpu.VMEM((2 * HKV, 8, DH), jnp.float32),
                pltpu.VMEM((2 * HKV, 8, DH), jnp.float32),
                pltpu.SemaphoreType.DMA((NBUF,)),
                pltpu.SemaphoreType.DMA((2,)),
                pltpu.SemaphoreType.DMA((2,)),
                pltpu.SemaphoreType.DMA((2 * NG,)),
            ],
            compiler_params=pltpu.CompilerParams(vmem_limit_bytes=100 * 2**20, disable_bounds_checks=nobc, disable_semaphore_checks=nosem, flags=flags),
        )(A_x.reshape(B, D), A_k_cache.reshape(-1, DH), A_v_cache.reshape(-1, DH), A_wq, A_wo.T,
          B_x.reshape(B, D), B_k_cache.reshape(-1, DH), B_v_cache.reshape(-1, DH), B_wq, B_wo.T)
        return out.reshape(B, 1, 2 * D)
    return f


@jax.jit
def pallas_concat_heads__gqa_block_cached__sliding_block_cached__decode_kernel(
    A_x, A_k_cache, A_v_cache, A_wq, A_wo, B_x, B_k_cache, B_v_cache, B_wq, B_wo):
    return make(tail=1,WQS=4)(A_x, A_k_cache, A_v_cache, A_wq, A_wo, B_x, B_k_cache, B_v_cache, B_wq, B_wo)
```

```python
import functools

import jax
import jax.numpy as jnp
from jax import lax
import jax.experimental.pallas as pl
import jax.experimental.pallas.tpu as pltpu

B, D, HQ, HKV, DH = 2, 448, 16, 8, 256
HD = HQ * DH
LOG2E = 1.4426950408889634
NT = (((1,), (1,)), ((), ()))

R = 2048
C = 64
WC = 2048
STREAMS = 4
LOOK = 4
NBUF = 6
TAIL = 4

SEM_WQ, SEM_X = 0, 2
SEM_A0, SEM_B0, SEM_A1, SEM_B1, SEM_A2, SEM_TAIL = range(6)


def _aligned(x, n):
    return x if isinstance(x, int) else pl.multiple_of(x, n)


def _wait_filled(dst, sem):
    pltpu.make_async_copy(dst, dst, sem).wait()


def _kernel(ax, ak, av, awq, awo, bx, bk, bv, bwq, bwo, out,
            kv, x_buf, wq_buf, wo_buf, q_scr, o_scr, kv_sem, w_sem):
    sk = ak.shape[0] // (B * HKV)
    window = min(4096, max(256, sk // 4))
    assert sk % R == 0 and window == R
    chunks = sk // R
    steps_a = B * HKV * chunks
    steps = steps_a + B * HKV

    def start_kv(k, v, src, slot, dst):
        src, dst = pl.ds(_aligned(src, C), C), pl.ds(_aligned(dst, C), C)
        pltpu.make_async_copy(k.at[src], kv.at[slot, 0, dst], kv_sem.at[slot]).start(priority=0)
        pltpu.make_async_copy(v.at[src], kv.at[slot, 1, dst], kv_sem.at[slot]).start(priority=1)

    def start_a(u, part=0, parts=1):
        seg = R // STREAMS
        base = (u // chunks) * sk + (u % chunks) * seg
        n = seg // C // parts
        for i in range(part * n, (part + 1) * n):
            for s in range(STREAMS):
                start_kv(ak, av, base + s * (sk // STREAMS) + i * C, u % NBUF, s * seg + i * C)

    def start_b(u):
        odd = (u - steps_a) % 2
        for i in range(R // 4 // C):
            for e in range(2):
                step_idx = u - odd + e
                for s in range(2):
                    r = s * (R // 2) + odd * (R // 4) + i * C
                    src = (step_idx - steps_a) * sk + (sk - window) + r
                    start_kv(bk, bv, src, step_idx % NBUF, r)

    def start_wq(j):
        for c in range(HD // WC):
            for s in range(STREAMS):
                rows = pl.ds(_aligned(s * (D // STREAMS) + j * 8, 8), 8)
                cols = pl.ds(c * WC, WC)
                for i, w in enumerate((awq, bwq)):
                    pltpu.make_async_copy(
                        w.at[rows, cols], wq_buf.at[i, rows, cols], w_sem.at[SEM_WQ + i]
                    ).start(priority=i)

    def start_wo(i, r, nr, c, nc, sem, priority):
        cols = pl.ds(c, nc)
        pltpu.make_async_copy(
            (awo, bwo)[i].at[pl.ds(_aligned(r, 8), nr), cols],
            wo_buf.at[pl.ds(_aligned(i * D + r, 8), nr), cols],
            w_sem.at[sem],
        ).start(priority=priority)

    def start_wo_head(u):
        assert 8 % LOOK == 0
        n = 0
        for j in range(8 // LOOK):
            r = ((u - steps) * (8 // LOOK) + j) * 8
            for c in range(HD // WC):
                for i, r0 in ((0, 0), (1, 0), (0, 64), (1, 64), (0, 128), (1, 128), (0, 192)):
                    start_wo(i, r0 + r, 8, c * WC, WC, (SEM_A0, SEM_B0)[i], n % 2)
                    n += 1

    x_copies = [pltpu.make_async_copy(x, x_buf.at[i], w_sem.at[SEM_X + i])
                for i, x in enumerate((ax, bx))]
    start_wq(0)
    for copy in x_copies:
        copy.start()
    lax.fori_loop(1, D // STREAMS // 8, lambda j, _: start_wq(j), None)
    lax.fori_loop(0, LOOK - 2, lambda u, _: start_a(u), None)

    row = lax.broadcasted_iota(jnp.int32, (8, DH), 0)
    o_scr[...] = jnp.zeros(o_scr.shape, o_scr.dtype)
    for i in range(2):
        x_copies[i].wait()
        x = x_buf[i].astype(jnp.float32)
        x_row = lax.broadcasted_iota(jnp.int32, (8, D), 0)
        x8 = jnp.where(x_row % 2 == 0, x[0:1, :], x[1:2, :]).astype(jnp.bfloat16)
        _wait_filled(wq_buf.at[i], w_sem.at[SEM_WQ + i])

        def project_q(h, _, i=i, x8=x8):
            cols = pl.ds(pl.multiple_of(h * 2 * DH, 2 * DH), 2 * DH)
            q2 = jnp.dot(x8, wq_buf[i, :, cols], preferred_element_type=jnp.float32)
            q_scr[i * HKV + h] = jnp.where(row % 4 < 2, q2[:, :DH], q2[:, DH:])

        for half in range(2):
            lax.fori_loop(half * HKV // 2, (half + 1) * HKV // 2, project_q, None)
            start_a(LOOK - 2 + i, half, 2)

    def step(start_ahead, t, carry):
        m, l, acc = carry
        slot = t % NBUF
        in_a = t < steps_a
        branch = jnp.where(in_a, 0, 1)
        bh = jnp.where(in_a, t // chunks, t - steps_a)
        chunk = jnp.where(in_a, t % chunks, 0)
        first = chunk == 0
        last = chunk == jnp.where(in_a, chunks - 1, 0)
        h = bh % HKV

        m = jnp.where(first, -jnp.inf, m)
        l = jnp.where(first, 0.0, l)
        acc = jnp.where(first, 0.0, acc)
        q = q_scr[branch * HKV + h].astype(jnp.bfloat16)
        _wait_filled(kv.at[slot], kv_sem.at[slot])

        s = lax.dot_general(q, kv[slot, 0], NT, preferred_element_type=jnp.float32)
        s = s * (LOG2E * DH ** -0.5)
        m_new = jnp.maximum(m, jnp.max(s, axis=1, keepdims=True))
        alpha = jnp.exp2(m - m_new)
        p = jnp.exp2(s - m_new)
        l = l * alpha + jnp.sum(p, axis=1, keepdims=True)
        acc = acc * alpha + jnp.dot(
            p.astype(jnp.bfloat16), kv[slot, 1], preferred_element_type=jnp.float32)
        start_ahead(t + LOOK)

        keep = jnp.logical_and((row & 5) == branch * 4 + bh // HKV, last)
        o_scr[h] = jnp.where(keep, acc / l, o_scr[h])
        return m_new, l, acc

    carry = (jnp.zeros((8, 1), jnp.float32), jnp.zeros((8, 1), jnp.float32),
             jnp.zeros((8, DH), jnp.float32))
    carry = lax.fori_loop(0, steps_a - LOOK, functools.partial(step, start_a), carry)
    carry = lax.fori_loop(steps_a - LOOK, steps - LOOK, functools.partial(step, start_b), carry)
    lax.fori_loop(steps - LOOK, steps, functools.partial(step, start_wo_head), carry)

    tail_cols = HD // TAIL
    tail_rows = 8 * WC // tail_cols
    blocks = lambda r0, segs: [(r0 + s * 64 + j * 8, 8, c * WC, WC)
                               for j in range(8) for c in range(HD // WC) for s in range(segs)]
    tail = [(1, 320 + s * 64 + j * tail_rows, tail_rows, c * tail_cols, tail_cols, SEM_TAIL + c)
            for c in range(TAIL) for j in range(64 // tail_rows) for s in range(2)]
    queue0 = ([(0, *blk, SEM_A1) for blk in blocks(256, 2)]
              + [(0, *blk, SEM_A2) for blk in blocks(384, 1)] + tail[:8])
    queue1 = [(1, *blk, SEM_B1) for blk in blocks(192, 2)] + tail[8:]
    pending = list(zip(queue0, queue1, strict=True))

    def start_pending(n):
        for _ in range(n):
            blk0, blk1 = pending.pop(0)
            start_wo(*blk0, 0)
            start_wo(*blk1, 1)

    def wait_wo(r0, r1, sem, c0=0, c1=HD):
        _wait_filled(wo_buf.at[pl.ds(r0, r1 - r0), pl.ds(c0, c1 - c0)], w_sem.at[sem])

    start_pending(len(pending) - 18)
    lhs = jnp.concatenate(
        [jnp.where(row // 2 % 2 == hq % 2, o_scr[hq // 2], 0.0).astype(jnp.bfloat16)
         for hq in range(HQ)], axis=1)

    def project_o(g, c0=0, c1=HD):
        return lax.dot_general(lhs[:, c0:c1], wo_buf[g * 128:(g + 1) * 128, c0:c1], NT,
                               preferred_element_type=jnp.float32)

    def write(g, y):
        ya, yb = y[0:2] + y[2:4], y[4:6] + y[6:8]
        if (g + 1) * 128 <= D:
            y = ya
        elif g * 128 >= D:
            y = yb
        else:
            y = jnp.where(lax.broadcasted_iota(jnp.int32, (B, 128), 1) < D - g * 128, ya, yb)
        out[:, g * 128:(g + 1) * 128] = y.astype(out.dtype)

    wait_wo(0, 256, SEM_A0)
    wait_wo(D, D + 192, SEM_B0)
    for g in (0, 1, 4):
        write(g, project_o(g))
        start_pending(6)
    assert not pending
    wait_wo(256, 384, SEM_A1)
    write(2, project_o(2))
    wait_wo(384, D, SEM_A2)
    write(3, project_o(3))
    wait_wo(D + 192, D + 320, SEM_B1)
    write(5, project_o(5))
    y = jnp.zeros((8, 128), jnp.float32)
    for c in range(TAIL):
        wait_wo(D + 320, 2 * D, SEM_TAIL + c, c * tail_cols, (c + 1) * tail_cols)
        y = y + project_o(6, c * tail_cols, (c + 1) * tail_cols)
    write(6, y)


@jax.jit
def pallas_concat_heads__gqa_block_cached__sliding_block_cached__decode_kernel(
    A_x: jax.Array,
    A_k_cache: jax.Array,
    A_v_cache: jax.Array,
    A_wq: jax.Array,
    A_wo: jax.Array,
    B_x: jax.Array,
    B_k_cache: jax.Array,
    B_v_cache: jax.Array,
    B_wq: jax.Array,
    B_wo: jax.Array,
):
    assert A_x.shape == B_x.shape == (B, 1, D)
    assert A_k_cache.shape == A_v_cache.shape == B_k_cache.shape == B_v_cache.shape
    assert A_k_cache.shape[:2] == (B, HKV) and A_k_cache.shape[3] == DH

    out = pl.pallas_call(
        _kernel,
        out_shape=jax.ShapeDtypeStruct((B, 2 * D), jnp.bfloat16),
        in_specs=[pl.BlockSpec(memory_space=pltpu.HBM)] * 10,
        out_specs=pl.BlockSpec(memory_space=pltpu.VMEM),
        scratch_shapes=[
            pltpu.VMEM((NBUF, 2, R, DH), jnp.bfloat16),
            pltpu.VMEM((2, B, D), jnp.bfloat16),
            pltpu.VMEM((2, D, HD), jnp.bfloat16),
            pltpu.VMEM((2 * D, HD), jnp.bfloat16),
            pltpu.VMEM((2 * HKV, 8, DH), jnp.float32),
            pltpu.VMEM((HKV, 8, DH), jnp.float32),
            pltpu.SemaphoreType.DMA((NBUF,)),
            pltpu.SemaphoreType.DMA((SEM_TAIL + TAIL,)),
        ],
        compiler_params=pltpu.CompilerParams(vmem_limit_bytes=48 * 2**20),
    )(
        A_x.reshape(B, D), A_k_cache.reshape(-1, DH), A_v_cache.reshape(-1, DH), A_wq, A_wo.T,
        B_x.reshape(B, D), B_k_cache.reshape(-1, DH), B_v_cache.reshape(-1, DH), B_wq, B_wo.T,
    )
    return out.reshape(B, 1, 2 * D)
```

```python
import functools

import jax
import jax.numpy as jnp
from jax import lax
import jax.experimental.pallas as pl
import jax.experimental.pallas.tpu as pltpu

B, D, HQ, HKV, DH = 2, 448, 16, 8, 256
HD = HQ * DH
LOG2E = 1.4426950408889634
NT = (((1,), (1,)), ((), ()))

R = 2048
C = 64
WC = 2048
STREAMS = 4
LOOK = 4
NBUF = 6
TAIL = 4

SEM_WQ, SEM_X = 0, 2
SEM_A0, SEM_B0, SEM_A1, SEM_B1, SEM_A2, SEM_TAIL = range(6)


def _aligned(x, n):
    return x if isinstance(x, int) else pl.multiple_of(x, n)


def _wait_filled(dst, sem):
    pltpu.make_async_copy(dst, dst, sem).wait()


def _kernel(ax, ak, av, awq, awo, bx, bk, bv, bwq, bwo, out,
            kv, x_buf, wq_buf, wo_buf, q_scr, o_scr, kv_sem, w_sem):
    sk = ak.shape[0] // (B * HKV)
    window = min(4096, max(256, sk // 4))
    assert sk % R == 0 and window == R
    chunks = sk // R
    steps_a = B * HKV * chunks
    steps = steps_a + B * HKV

    def start_kv(k, v, src, slot, dst):
        src, dst = pl.ds(_aligned(src, C), C), pl.ds(_aligned(dst, C), C)
        pltpu.make_async_copy(k.at[src], kv.at[slot, 0, dst], kv_sem.at[slot]).start(priority=0)
        pltpu.make_async_copy(v.at[src], kv.at[slot, 1, dst], kv_sem.at[slot]).start(priority=1)

    def start_a(u, part=0, parts=1):
        seg = R // STREAMS
        base = (u // chunks) * sk + (u % chunks) * seg
        n = seg // C // parts
        for i in range(part * n, (part + 1) * n):
            for s in range(STREAMS):
                start_kv(ak, av, base + s * (sk // STREAMS) + i * C, u % NBUF, s * seg + i * C)

    def start_b(u):
        odd = (u - steps_a) % 2
        for i in range(R // 4 // C):
            for e in range(2):
                step_idx = u - odd + e
                for s in range(2):
                    r = s * (R // 2) + odd * (R // 4) + i * C
                    src = (step_idx - steps_a) * sk + (sk - window) + r
                    start_kv(bk, bv, src, step_idx % NBUF, r)

    def start_wq(j, min_priority=0):
        for c in range(HD // WC):
            for s in range(STREAMS):
                rows = pl.ds(_aligned(s * (D // STREAMS) + j * 8, 8), 8)
                cols = pl.ds(c * WC, WC)
                for i, w in enumerate((awq, bwq)):
                    pltpu.make_async_copy(
                        w.at[rows, cols], wq_buf.at[i, rows, cols], w_sem.at[SEM_WQ + i]
                    ).start(priority=max(i, min_priority))

    def start_wo(i, r, nr, c, nc, sem, priority):
        cols = pl.ds(c, nc)
        pltpu.make_async_copy(
            (awo, bwo)[i].at[pl.ds(_aligned(r, 8), nr), cols],
            wo_buf.at[pl.ds(_aligned(i * D + r, 8), nr), cols],
            w_sem.at[sem],
        ).start(priority=priority)

    def start_wo_head(u):
        assert 8 % LOOK == 0
        n = 0
        for j in range(8 // LOOK):
            r = ((u - steps) * (8 // LOOK) + j) * 8
            for c in range(HD // WC):
                for i, r0 in ((0, 0), (1, 0), (0, 64), (1, 64), (0, 128), (1, 128), (0, 192)):
                    start_wo(i, r0 + r, 8, c * WC, WC, (SEM_A0, SEM_B0)[i], n % 2)
                    n += 1

    x_copies = [pltpu.make_async_copy(x, x_buf.at[i], w_sem.at[SEM_X + i])
                for i, x in enumerate((ax, bx))]
    start_wq(0, 1)
    for copy in x_copies:
        copy.start()
    start_wq(1, 1)
    lax.fori_loop(2, D // STREAMS // 8, lambda j, _: start_wq(j), None)
    lax.fori_loop(0, LOOK - 2, lambda u, _: start_a(u), None)

    row = lax.broadcasted_iota(jnp.int32, (8, DH), 0)
    o_scr[...] = jnp.zeros(o_scr.shape, o_scr.dtype)
    for i in range(2):
        x_copies[i].wait()
        x = x_buf[i].astype(jnp.float32)
        x_row = lax.broadcasted_iota(jnp.int32, (8, D), 0)
        x8 = jnp.where(x_row % 2 == 0, x[0:1, :], x[1:2, :]).astype(jnp.bfloat16)
        _wait_filled(wq_buf.at[i], w_sem.at[SEM_WQ + i])

        def project_q(h, _, i=i, x8=x8):
            cols = pl.ds(pl.multiple_of(h * 2 * DH, 2 * DH), 2 * DH)
            q2 = jnp.dot(x8, wq_buf[i, :, cols], preferred_element_type=jnp.float32)
            q_scr[i * HKV + h] = jnp.where(row % 4 < 2, q2[:, :DH], q2[:, DH:])

        for half in range(2):
            lax.fori_loop(half * HKV // 2, (half + 1) * HKV // 2, project_q, None)
            start_a(LOOK - 2 + i, half, 2)

    def step(start_ahead, t, carry):
        m, l, acc = carry
        slot = t % NBUF
        in_a = t < steps_a
        branch = jnp.where(in_a, 0, 1)
        bh = jnp.where(in_a, t // chunks, t - steps_a)
        chunk = jnp.where(in_a, t % chunks, 0)
        first = chunk == 0
        last = chunk == jnp.where(in_a, chunks - 1, 0)
        h = bh % HKV

        m = jnp.where(first, -jnp.inf, m)
        l = jnp.where(first, 0.0, l)
        acc = jnp.where(first, 0.0, acc)
        q = q_scr[branch * HKV + h].astype(jnp.bfloat16)
        _wait_filled(kv.at[slot], kv_sem.at[slot])

        s = lax.dot_general(q, kv[slot, 0], NT, preferred_element_type=jnp.float32)
        s = s * (LOG2E * DH ** -0.5)
        m_new = jnp.maximum(m, jnp.max(s, axis=1, keepdims=True))
        alpha = jnp.exp2(m - m_new)
        p = jnp.exp2(s - m_new)
        l = l * alpha + jnp.sum(p, axis=1, keepdims=True)
        acc = acc * alpha + jnp.dot(
            p.astype(jnp.bfloat16), kv[slot, 1], preferred_element_type=jnp.float32)
        start_ahead(t + LOOK)

        keep = jnp.logical_and((row & 5) == branch * 4 + bh // HKV, last)
        o_scr[h] = jnp.where(keep, acc / l, o_scr[h])
        return m_new, l, acc

    carry = (jnp.zeros((8, 1), jnp.float32), jnp.zeros((8, 1), jnp.float32),
             jnp.zeros((8, DH), jnp.float32))
    carry = lax.fori_loop(0, steps_a - LOOK, functools.partial(step, start_a), carry)
    carry = lax.fori_loop(steps_a - LOOK, steps - LOOK, functools.partial(step, start_b), carry)
    lax.fori_loop(steps - LOOK, steps, functools.partial(step, start_wo_head), carry)

    tail_cols = HD // TAIL
    tail_rows = 8 * WC // tail_cols
    blocks = lambda r0, segs: [(r0 + s * 64 + j * 8, 8, c * WC, WC)
                               for j in range(8) for c in range(HD // WC) for s in range(segs)]
    tail = [(1, 320 + s * 64 + j * tail_rows, tail_rows, c * tail_cols, tail_cols, SEM_TAIL + c)
            for c in range(TAIL) for j in range(64 // tail_rows) for s in range(2)]
    queue0 = ([(0, *blk, SEM_A1) for blk in blocks(256, 2)]
              + [(0, *blk, SEM_A2) for blk in blocks(384, 1)] + tail[:8])
    queue1 = [(1, *blk, SEM_B1) for blk in blocks(192, 2)] + tail[8:]
    pending = list(zip(queue0, queue1, strict=True))

    def start_pending(n):
        for _ in range(n):
            blk0, blk1 = pending.pop(0)
            start_wo(*blk0, 0)
            start_wo(*blk1, 1)

    def wait_wo(r0, r1, sem, c0=0, c1=HD):
        _wait_filled(wo_buf.at[pl.ds(r0, r1 - r0), pl.ds(c0, c1 - c0)], w_sem.at[sem])

    start_pending(len(pending) - 18)
    lhs = jnp.concatenate(
        [jnp.where(row // 2 % 2 == hq % 2, o_scr[hq // 2], 0.0).astype(jnp.bfloat16)
         for hq in range(HQ)], axis=1)

    def project_o(g, c0=0, c1=HD):
        return lax.dot_general(lhs[:, c0:c1], wo_buf[g * 128:(g + 1) * 128, c0:c1], NT,
                               preferred_element_type=jnp.float32)

    def write(g, y):
        ya, yb = y[0:2] + y[2:4], y[4:6] + y[6:8]
        if (g + 1) * 128 <= D:
            y = ya
        elif g * 128 >= D:
            y = yb
        else:
            y = jnp.where(lax.broadcasted_iota(jnp.int32, (B, 128), 1) < D - g * 128, ya, yb)
        out[:, g * 128:(g + 1) * 128] = y.astype(out.dtype)

    wait_wo(0, 256, SEM_A0)
    wait_wo(D, D + 192, SEM_B0)
    for g in (0, 1, 4):
        write(g, project_o(g))
        start_pending(6)
    assert not pending
    wait_wo(256, 384, SEM_A1)
    write(2, project_o(2))
    wait_wo(384, D, SEM_A2)
    write(3, project_o(3))
    wait_wo(D + 192, D + 320, SEM_B1)
    write(5, project_o(5))
    y = jnp.zeros((8, 128), jnp.float32)
    for c in range(TAIL):
        wait_wo(D + 320, 2 * D, SEM_TAIL + c, c * tail_cols, (c + 1) * tail_cols)
        y = y + project_o(6, c * tail_cols, (c + 1) * tail_cols)
    write(6, y)


@jax.jit
def pallas_concat_heads__gqa_block_cached__sliding_block_cached__decode_kernel(
    A_x: jax.Array,
    A_k_cache: jax.Array,
    A_v_cache: jax.Array,
    A_wq: jax.Array,
    A_wo: jax.Array,
    B_x: jax.Array,
    B_k_cache: jax.Array,
    B_v_cache: jax.Array,
    B_wq: jax.Array,
    B_wo: jax.Array,
):
    assert A_x.shape == B_x.shape == (B, 1, D)
    assert A_k_cache.shape == A_v_cache.shape == B_k_cache.shape == B_v_cache.shape
    assert A_k_cache.shape[:2] == (B, HKV) and A_k_cache.shape[3] == DH

    out = pl.pallas_call(
        _kernel,
        out_shape=jax.ShapeDtypeStruct((B, 2 * D), jnp.bfloat16),
        in_specs=[pl.BlockSpec(memory_space=pltpu.HBM)] * 10,
        out_specs=pl.BlockSpec(memory_space=pltpu.VMEM),
        scratch_shapes=[
            pltpu.VMEM((NBUF, 2, R, DH), jnp.bfloat16),
            pltpu.VMEM((2, B, D), jnp.bfloat16),
            pltpu.VMEM((2, D, HD), jnp.bfloat16),
            pltpu.VMEM((2 * D, HD), jnp.bfloat16),
            pltpu.VMEM((2 * HKV, 8, DH), jnp.float32),
            pltpu.VMEM((HKV, 8, DH), jnp.float32),
            pltpu.SemaphoreType.DMA((NBUF,)),
            pltpu.SemaphoreType.DMA((SEM_TAIL + TAIL,)),
        ],
        compiler_params=pltpu.CompilerParams(vmem_limit_bytes=48 * 2**20),
    )(
        A_x.reshape(B, D), A_k_cache.reshape(-1, DH), A_v_cache.reshape(-1, DH), A_wq, A_wo.T,
        B_x.reshape(B, D), B_k_cache.reshape(-1, DH), B_v_cache.reshape(-1, DH), B_wq, B_wo.T,
    )
    return out.reshape(B, 1, 2 * D)
```
